```python
import os as _os
_os.environ.setdefault('JAX_PLATFORMS', 'cpu')
import jax
import jax.numpy as jnp

def _softmax(x, axis=-1):
    return jax.nn.softmax(x, axis=axis)

def _gelu(x):
    return jax.nn.gelu(x, approximate=True)

def _silu(x):
    return jax.nn.silu(x)

def _sigmoid(x):
    return jax.nn.sigmoid(x)

def _layernorm(x, axis=-1, eps=1e-05):
    m = jnp.mean(x, axis=axis, keepdims=True)
    v = jnp.var(x, axis=axis, keepdims=True)
    return (x - m) / jnp.sqrt(v + eps)

def _scatter_add(tgt, idx, src, axis=0):
    return tgt.at[idx].add(src)

def _segment_sum(src, seg, n):
    return jax.ops.segment_sum(src, seg, n)

class _Rng:

    def __init__(self, key):
        self._k = key

    def _next(self):
        self._k, sub = jax.random.split(self._k)
        return sub

    def normal(self, shape):
        return jax.random.normal(self._next(), shape, dtype=jnp.bfloat16)

    def randint(self, lo, hi, shape):
        return jax.random.randint(self._next(), shape, lo, hi, dtype=jnp.int32)

    def uniform(self, shape, lo=0.0, hi=1.0):
        return jax.random.uniform(self._next(), shape, jnp.bfloat16, lo, hi)

    def permutation(self, n):
        return jax.random.permutation(self._next(), n)
kernel_name = 'adaLN_cond__mha_block__geglu_ffn__prompt'

def setup_inputs():
    _rng = _Rng(jax.random.key(int.from_bytes(__import__("os").urandom(4), "little")))
    _w = lambda a: (lambda t: t.astype(jnp.bfloat16) if jnp.issubdtype(t.dtype, jnp.floating) else t)(jnp.asarray(a))

    def _A_setup():
        B, S, D, H = (1, 2048, 640, 32)
        return {'x': _w((lambda *s: _rng.normal(s) * 0.05)(B, S, D)), 'wqkv': _w((lambda *s: _rng.normal(s) * 0.05)(D, 3 * D)), 'wo': _w((lambda *s: _rng.normal(s) * 0.05)(D, D))}
    _A_in = _A_setup()

    def _B_setup():
        B, S, D, F = (1, 2048, 640, 1728)
        return {'x': _w((lambda *s: _rng.normal(s) * 0.05)(B, S, D)), 'w_gate': _w((lambda *s: _rng.normal(s) * 0.05)(D, F)), 'w_up': _w((lambda *s: _rng.normal(s) * 0.05)(D, F)), 'w_down': _w((lambda *s: _rng.normal(s) * 0.05)(F, D))}
    _B_in = _B_setup()
    return {'A_x': _A_in['x'], 'A_wqkv': _A_in['wqkv'], 'A_wo': _A_in['wo'], 'B_x': _B_in['x'], 'B_w_gate': _B_in['w_gate'], 'B_w_up': _B_in['w_up'], 'B_w_down': _B_in['w_down'], 'c': _w((lambda *s: _rng.normal(s) * 0.05)(1, 640) * 8.0), 'w_mod': _w((lambda *s: _rng.normal(s) * 0.05)(640, 6 * 640) * 640 ** (-0.5) * 8.0)}

def reference(A_x, A_wqkv, A_wo, B_x, B_w_gate, B_w_up, B_w_down, c, w_mod):

    def _A_ref(x, wqkv, wo):
        B, S, D = x.shape
        H = 32
        Dh = D // H
        qkv = (lambda x, *d: x.transpose(*d))((x @ wqkv).reshape(B, S, 3, H, Dh), 2, 0, 3, 1, 4)
        q, k, v = (qkv[0], qkv[1], qkv[2])
        scores = jnp.einsum('bhqd,bhkd->bhqk', q, k) * Dh ** (-0.5)
        p = _softmax(scores, axis=-1)
        o = jnp.einsum('bhqk,bhkd->bhqd', p, v)
        return (lambda x, *d: x.transpose(*d))(o, 0, 2, 1, 3).reshape(B, S, D) @ wo

    def _B_ref(x, w_gate, w_up, w_down):
        return _gelu(x @ w_gate) * (x @ w_up) @ w_down
    x = A_x
    mod = (_silu(c) @ w_mod).reshape(c.shape[0], 6, 1, -1)
    sa, ca, ga, sb, cb, gb = (mod[:, 0].copy(), mod[:, 1].copy(), mod[:, 2].copy(), mod[:, 3].copy(), mod[:, 4].copy(), mod[:, 5].copy())
    h = _layernorm(x, axis=-1) * (1 + ca) + sa
    x = x + ga * _A_ref(h, A_wqkv, A_wo)
    h = _layernorm(x, axis=-1) * (1 + cb) + sb
    x = x + gb * _B_ref(h, B_w_gate, B_w_up, B_w_down)
    return x
```

```python
import math

import jax
import jax.numpy as jnp
from jax import lax
import jax.experimental.pallas as pl
import jax.experimental.pallas.tpu as pltpu

_H = 32
_LANES = 128
_RB = 512
_KB = 128
_GROUP = 4
_FB = 256
_VROWS = 24
_EPS = 1e-5

_F32 = jnp.float32
_BF16 = jnp.bfloat16
_NT = (((1,), (1,)), ((), ()))


def _dot(a, b):
  return jnp.dot(a, b, preferred_element_type=_F32)


def _dot_nt(a, b):
  return lax.dot_general(a, b, _NT, preferred_element_type=_F32)


def _layernorm(x):
  mean = jnp.mean(x, axis=-1, keepdims=True)
  xc = x - mean
  var = jnp.mean(xc * xc, axis=-1, keepdims=True)
  return xc * lax.rsqrt(var + _EPS)


def _gelu(x):
  c = math.sqrt(2.0 / math.pi)
  inner = x * (c + (c * 0.044715) * (x * x))
  half = 0.5 * x
  return half + half * jnp.tanh(inner)


def _kernel(x_hbm, wqkv_hbm, wo_hbm, wg_hbm, wu_hbm, wd_hbm, c_hbm, wmod_hbm,
            out_hbm,
            x_v, wqkv_v, wo_v, wgu_v, wd_v, c_v, wmod_v, out_v,
            wqv_t, k_tiles, q_tiles, v_t, s_buf, r_buf, o_t, mod_v,
            sems, out_sems):
  seq, d = x_v.shape
  f = wd_v.shape[0]
  dh = d // _H
  n_dt = d // _LANES
  n_rb = seq // _RB
  f_main = (f // _LANES) * _LANES
  f_tail = f - f_main

  def cols(ref, lo, hi):
    return ref.at[:, pl.ds(lo, hi - lo)]

  def rows(ref, lo, hi):
    return ref.at[pl.ds(lo, hi - lo), :]

  pairs = dict(
      c=(c_hbm, c_v),
      mod_a=(cols(wmod_hbm, 0, 2 * d), cols(wmod_v, 0, 2 * d)),
      x0=(rows(x_hbm, 0, _RB), rows(x_v, 0, _RB)),
      wk=(cols(wqkv_hbm, d, 2 * d), cols(wqkv_v, d, 2 * d)),
      wq=(cols(wqkv_hbm, 0, d), cols(wqkv_v, 0, d)),
      wv=(cols(wqkv_hbm, 2 * d, 3 * d), cols(wqkv_v, 2 * d, 3 * d)),
      x1=(rows(x_hbm, _RB, seq), rows(x_v, _RB, seq)),
      mod_b=(cols(wmod_hbm, 2 * d, 6 * d), cols(wmod_v, 2 * d, 6 * d)),
      wo=(wo_hbm, wo_v),
      wg=(rows(wg_hbm, 0, f_main), rows(wgu_v, 0, f_main)),
      wu=(rows(wu_hbm, 0, f_main), rows(wgu_v, f_main, 2 * f_main)),
      wg_tail=(rows(wg_hbm, f_main, f),
               rows(wgu_v, 2 * f_main, 2 * f_main + f_tail)),
      wu_tail=(rows(wu_hbm, f_main, f), rows(wgu_v, 2 * f_main + f_tail, 2 * f)),
      wd=(wd_hbm, wd_v),
  )
  copies = {
      name: pltpu.make_async_copy(src, dst, sems.at[i])
      for i, (name, (src, dst)) in enumerate(pairs.items())
  }

  late = ("mod_b", "wo", "wg", "wu", "wg_tail", "wu_tail", "wd")

  for name in ("c", "mod_a", "x0", "wk"):
    copies[name].start()
  copies["c"].wait()
  copies["mod_a"].wait()
  for name in ("wq", "wv", "x1"):
    copies[name].start()

  c32 = c_v[...].astype(_F32)
  silu_c = jnp.broadcast_to(c32 * jax.nn.sigmoid(c32), (16, d)).astype(_BF16)
  mod_a = _dot(silu_c, wmod_v[:, 0:2 * d])
  shift_a = mod_a[0:1, 0:d]
  scale_a = 1.0 + mod_a[0:1, d:2 * d]

  q_scale = dh ** -0.5 * math.log2(math.e)
  lane_hi = lax.broadcasted_iota(jnp.int32, (_RB, _LANES), 1) >= _LANES // 2
  sub8 = lax.broadcasted_iota(jnp.int32, (8, _RB), 0)

  def adaln_a(b):
    xb = x_v[pl.ds(b * _RB, _RB), :].astype(_F32)
    return (_layernorm(xb) * scale_a + shift_a).astype(_BF16)

  def project_k(b, h):
    r = pl.ds(b * _RB, _RB)
    k = _dot(h, wqkv_v[:, d:2 * d])
    tiles = [k[:, t * _LANES:(t + 1) * _LANES] for t in range(n_dt)]
    for t in range(n_dt):
      k_tiles[t, r, :] = tiles[t].astype(_BF16)
    for t in range(n_dt - 1):
      k_tiles[n_dt + t, r, :] = jnp.where(
          lane_hi, tiles[t], tiles[t + 1]).astype(_BF16)

  def project_qv(b, h):
    qv = _dot_nt(wqv_t[...], h)
    q = (qv[0:d] * q_scale).astype(_BF16)
    half = _LANES // 2
    for t in range(n_dt):
      q_tiles[b, t] = q[t * _LANES:(t + 1) * _LANES]
    for t in range(n_dt - 1):
      edge = (t + 1) * _LANES
      q_tiles[b, n_dt + t, 0:half, :] = q[edge:edge + half]
      q_tiles[b, n_dt + t, half:_LANES, :] = q[edge - half:edge]
    v = qv[d:2 * d].astype(_BF16).astype(_F32)
    r = pl.ds(b * _RB, _RB)
    for pair in range(_H // 2):
      base = pair * 2 * dh
      shared = v[base + 16:base + 24]
      v_t[2 * pair, 0:16, r] = v[base:base + 16]
      v_t[2 * pair, 16:24, r] = jnp.where(sub8 < 4, shared, 1.0)
      v_t[2 * pair + 1, 0:8, r] = jnp.where(sub8 < 4, 1.0, shared)
      v_t[2 * pair + 1, 8:24, r] = v[base + 24:base + 40]

  copies["x0"].wait()
  h0 = adaln_a(0)
  copies["wk"].wait()
  project_k(0, h0)
  copies["wq"].wait()
  copies["wv"].wait()
  copies["x1"].wait()
  for name in late:
    copies[name].start()
  wqv_t[0:d, :] = wqkv_v[:, 0:d].T
  wqv_t[d:2 * d, :] = wqkv_v[:, 2 * d:3 * d].T
  project_qv(0, h0)
  for b in range(1, n_rb):
    h = adaln_a(b)
    project_k(b, h)
    project_qv(b, h)

  n_kb = seq // _KB
  pair_row = lax.broadcasted_iota(jnp.int32, (_LANES // 2, _RB), 0)

  def head_tile(head):
    lo = head * dh
    t_lo = lo // _LANES
    t_hi = (lo + dh - 1) // _LANES
    return jnp.where(t_lo == t_hi, t_lo, n_dt + t_lo)

  def load_queries(slot, qb, head, tile):
    q = pltpu.bitcast(q_tiles[qb, tile], jnp.uint32)
    mine = ((pair_row - head * (dh // 2)) & (_LANES // 2 - 1)) < dh // 2
    r_buf[slot] = pltpu.bitcast(jnp.where(mine, q, jnp.uint32(0)), _BF16)

  def scores(slot, tile, j):
    r = pl.ds(j * _KB, _KB)
    return _dot(k_tiles[tile, r, :], r_buf[slot])

  def fold_max(mx, s):
    m = jnp.max(s.reshape(_KB // 8, 8, _RB), axis=0)
    return m if mx is None else jnp.maximum(mx, m)

  def weighted_values(head, m, j):
    r = pl.ds(j * _KB, _KB)
    p = jnp.exp2(s_buf[r, :] - m).astype(_BF16)
    return _dot(v_t[head, :, r], p)

  def attend(cur, nxt, m):
    acc = mx = None
    if nxt is not None:
      slot, qb, head = nxt
      tile = head_tile(head)
      load_queries(slot, qb, head, tile)
    for j in range(n_kb):
      if nxt is not None:
        s = scores(slot, tile, j)
      if cur is not None:
        o = weighted_values(cur, m, j)
        acc = o if acc is None else acc + o
      if nxt is not None:
        s_buf[pl.ds(j * _KB, _KB), :] = s
        mx = fold_max(mx, s)
    if nxt is not None:
      m = jnp.max(mx, axis=0, keepdims=True)
    return acc, m

  def normalise_pair(even, odd):
    even = even * (1.0 / even[20:21])
    odd = odd * (1.0 / odd[0:1])
    shared = jnp.where(sub8 < 4, even[16:24], odd[0:8])
    return [even[0:16], shared, odd[8:24]]

  n_groups = _H // _GROUP

  def group(i, m, last=False):
    qb = i // n_groups
    g = i % n_groups
    accs = []
    for u in range(_GROUP):
      head = g * _GROUP + u
      if u + 1 < _GROUP:
        nxt = ((u + 1) % _GROUP, qb, head + 1)
      elif last:
        nxt = None
      else:
        nxt = (0, (i + 1) // n_groups, ((i + 1) % n_groups) * _GROUP)
      acc, m = attend(head, nxt, m)
      accs.append(acc)
    parts = []
    for u in range(0, _GROUP, 2):
      parts += normalise_pair(accs[u], accs[u + 1])
    row0 = g * _GROUP * dh
    if not isinstance(row0, int):
      row0 = pl.multiple_of(row0, 16)
    o_t[qb, pl.ds(row0, _GROUP * dh), :] = jnp.concatenate(
        parts, axis=0).astype(_BF16)
    return m

  _, m0 = attend(None, (0, 0, 0), None)
  n_iter = n_rb * n_groups
  m_last = lax.fori_loop(0, n_iter - 1, group, m0)
  group(n_iter - 1, m_last, last=True)

  for name in late:
    copies[name].wait()
  mod_v[...] = _dot(silu_c, wmod_v[:, 2 * d:6 * d])[0:8]

  def out_copy(b):
    r = pl.ds(b * _RB, _RB)
    return pltpu.make_async_copy(
        out_v.at[r, :], out_hbm.at[r, :], out_sems.at[b])

  def residual_a(b, part):
    gate_a = mod_v[0:1, 0:d]
    shift_b = mod_v[0:1, d:2 * d]
    scale_b = 1.0 + mod_v[0:1, 2 * d:3 * d]
    r = pl.ds(pl.multiple_of(b * _RB, _RB) + part * _FB, _FB)
    o = o_t[b, :, pl.ds(part * _FB, _FB)].T
    x1 = x_v[r, :].astype(_F32) + gate_a * _dot(o, wo_v[...])
    return x1, (_layernorm(x1) * scale_b + shift_b).astype(_BF16)

  def ffn(b, part, x1, h):
    gate_b = mod_v[0:1, 3 * d:4 * d]
    r = pl.ds(pl.multiple_of(b * _RB, _RB) + part * _FB, _FB)
    act = _gelu(_dot_nt(h, wgu_v[0:f_main, :])) * _dot_nt(
        h, wgu_v[f_main:2 * f_main, :])
    tail = _dot_nt(h, wgu_v[2 * f_main:2 * f, :])
    act_tail = _gelu(tail[:, 0:f_tail]) * tail[:, f_tail:2 * f_tail]
    y = _dot(act.astype(_BF16), wd_v[0:f_main, :])
    y = y + _dot(act_tail.astype(_BF16), wd_v[f_main:f, :])
    out_v[r, :] = (x1 + gate_b * y).astype(out_v.dtype)

  def post_block(b, _):
    pre = [residual_a(b, part) for part in range(_RB // _FB)]
    for part, (x1, h) in enumerate(pre):
      ffn(b, part, x1, h)
    out_copy(b).start()
    return 0

  lax.fori_loop(0, n_rb, post_block, 0)
  for b in range(n_rb):
    out_copy(b).wait()


@jax.jit
def pallas_adaLN_cond__mha_block__geglu_ffn__prompt_kernel(
    A_x: jax.Array,
    A_wqkv: jax.Array,
    A_wo: jax.Array,
    B_x: jax.Array,
    B_w_gate: jax.Array,
    B_w_up: jax.Array,
    B_w_down: jax.Array,
    c: jax.Array,
    w_mod: jax.Array,
):
  del B_x
  batch, seq, d = A_x.shape
  assert batch == 1 and d == _H * 20
  n_dt = d // _LANES
  n_rb = seq // _RB

  def like(a):
    return pltpu.VMEM(a.shape, a.dtype)

  out = pl.pallas_call(
      _kernel,
      out_shape=jax.ShapeDtypeStruct((seq, d), A_x.dtype),
      in_specs=[pl.BlockSpec(memory_space=pltpu.HBM)] * 8,
      out_specs=pl.BlockSpec(memory_space=pltpu.HBM),
      scratch_shapes=[
          pltpu.VMEM((seq, d), A_x.dtype),
          like(A_wqkv), like(A_wo),
          pltpu.VMEM((2 * B_w_down.shape[0], d), B_w_gate.dtype),
          like(B_w_down), like(c), like(w_mod),
          pltpu.VMEM((seq, d), A_x.dtype),
          pltpu.VMEM((2 * d, d), _BF16),
          pltpu.VMEM((2 * n_dt - 1, seq, _LANES), _BF16),
          pltpu.VMEM((n_rb, 2 * n_dt - 1, _LANES, _RB), _BF16),
          pltpu.VMEM((_H, _VROWS, seq), _F32),
          pltpu.VMEM((seq, _RB), _F32),
          pltpu.VMEM((_GROUP, _LANES, _RB), _BF16),
          pltpu.VMEM((n_rb, d, _RB), _BF16),
          pltpu.VMEM((8, 4 * d), _F32),
          pltpu.SemaphoreType.DMA((14,)),
          pltpu.SemaphoreType.DMA((n_rb,)),
      ],
      compiler_params=pltpu.CompilerParams(
          vmem_limit_bytes=100 * 1024 * 1024),
      name="adaln_mha_geglu",
  )(A_x.reshape(seq, d), A_wqkv, A_wo, B_w_gate.T, B_w_up.T, B_w_down, c,
    w_mod)
  return out.reshape(batch, seq, d)
```

```python
import math

import jax
import jax.numpy as jnp
from jax import lax
import jax.experimental.pallas as pl
import jax.experimental.pallas.tpu as pltpu

_HEADS = 32
_DH = 20
_LANES = 128
_QB = 512
_NT = _QB // _LANES
_RB = _QB // 2
_KB = 128
_VK = 16
_NB = _KB // _VK
_VROWS = 24
_VPU_AT = (0, 4, 2, 6)
_PERIOD = 8
_EXTRA = 2
_EXTRA_AT = 5
_SPLAT = 6
_STRASSEN_K = 2 * _LANES
_EPS = 1e-5
_SAFE_LO = 2.0 ** -60
_SAFE_HI = 2.0 ** 60

_F32 = jnp.float32
_BF16 = jnp.bfloat16
_U32 = jnp.uint32


def _dot(a, b):
  return jnp.dot(a, b, preferred_element_type=_F32)


def _dot_nt(a, b):
  return lax.dot_general(a, b, (((1,), (1,)), ((), ())),
                         preferred_element_type=_F32)


def _pack(x):
  return pltpu.bitcast(x.astype(_BF16), _U32)


def _unpack(x):
  return pltpu.bitcast(x, _BF16)


def _aligned(i, n):
  return i if isinstance(i, int) else pl.multiple_of(i, n)


def _layernorm(x):
  mean = jnp.mean(x, axis=-1, keepdims=True)
  centred = x - mean
  var = jnp.mean(centred * centred, axis=-1, keepdims=True)
  return centred * lax.rsqrt(var + _EPS)


def _gelu(x):
  c = math.sqrt(2.0 / math.pi)
  half = 0.5 * x
  return half + half * jnp.tanh(x * (c + (c * 0.044715) * (x * x)))


def _strassen_lhs(a11, a12, a21, a22):
  return [a.astype(_BF16) for a in (
      a11 + a22, a21 + a22, a11, a22, a11 + a12, a21 - a11, a12 - a22)]


def _strassen_rhs_sums(b11, b12, b21, b22):
  b11, b12, b21, b22 = [b.astype(_F32) for b in (b11, b12, b21, b22)]
  return [b.astype(_BF16) for b in (
      b11 + b22, b12 - b22, b21 - b11, b11 + b12, b21 + b22)]


def _strassen(dot, lhs, sums, b11, b22, init=None):
  rhs = [sums[0], b11, sums[1], sums[2], b22, sums[3], sums[4]]
  signs = ((1, 0, 0, 1), (0, 0, 1, -1), (0, 1, 0, 1), (1, 0, 1, 0),
           (-1, 1, 0, 0), (0, 0, 0, 1), (1, 0, 0, 0))
  c = [None] * 4
  if init is not None:
    c = [q for row in zip(*[jnp.split(x, 2) for x in init]) for q in row]
  for n in (2, 4, 1, 3, 0, 6, 5):
    m = dot(lhs[n], rhs[n])
    for i, sign in enumerate(signs[n]):
      if sign and c[i] is None:
        c[i] = m if sign > 0 else -m
      elif sign:
        c[i] = c[i] + m if sign > 0 else c[i] - m
  return jnp.concatenate([c[0], c[2]]), jnp.concatenate([c[1], c[3]])


def _kernel(
    x_hbm, wqkv_hbm, wo_hbm, wg_hbm, wu_hbm, wd_hbm, c_hbm, wmod_hbm, out_hbm,
    x_v, wqkv_v, wo_v, wgu_v, wd_v, wmod_v, c_v, out_v,
    mod_v, wqv_t, h_v, k_mxu, k_vpu, splat_even, splat_odd, q_mxu, q_vpu, v_t,
    p_first, o_t, unsafe_v, o_v, act_v, wgu_sums, wd_sums, zeros_s,
    sems, out_sems):
  seq, d = x_v.shape
  f = wd_hbm.shape[0]
  n_qb = seq // _QB
  n_steps = seq // _KB
  n_vpu = n_steps + n_steps // _PERIOD
  rb_steps = _RB // _KB
  n_pairs = _HEADS // 2
  pd = 2 * _DH
  f_main = f // _LANES * _LANES
  f_tail = f - f_main
  sk = _STRASSEN_K
  fh = wd_sums.shape[1]

  def cols(src, dst, lo, hi):
    return src.at[:, pl.ds(lo, hi - lo)], dst.at[:, pl.ds(lo, hi - lo)]

  def rows(src, dst, lo, hi, to=None):
    return (src.at[pl.ds(lo, hi - lo), :],
            dst.at[pl.ds(lo if to is None else to, hi - lo), :])

  pieces = dict(
      c=(c_hbm, c_v.at[0]),
      x0=rows(x_hbm, x_v, 0, _QB),
      shift=cols(wmod_hbm, wmod_v, 0, d),
      scale=cols(wmod_hbm, wmod_v, d, 2 * d),
      wk=cols(wqkv_hbm, wqkv_v, d, 2 * d),
      wq=cols(wqkv_hbm, wqkv_v, 0, d),
      wv=cols(wqkv_hbm, wqkv_v, 2 * d, 3 * d),
      x1=rows(x_hbm, x_v, _QB, _QB + _RB),
      x2=rows(x_hbm, x_v, _QB + _RB, seq),
      mod=cols(wmod_hbm, wmod_v, 2 * d, 6 * d),
      wo=(wo_hbm, wo_v),
      wg=rows(wg_hbm, wgu_v, 0, f_main),
      wu=rows(wu_hbm, wgu_v, 0, f_main, f_main),
      wg_tail=rows(wg_hbm, wgu_v, f_main, f, 2 * f_main),
      wu_tail=rows(wu_hbm, wgu_v, f_main, f, 2 * f_main + f_tail),
      wd=rows(wd_hbm, wd_v, 0, f),
  )
  copies = {name: pltpu.make_async_copy(src, dst, sems.at[i])
            for i, (name, (src, dst)) in enumerate(pieces.items())}
  late = ("mod", "wo", "wg", "wu", "wg_tail", "wu_tail", "wd")

  def start(*names):
    for name in names:
      copies[name].start()

  def wait(*names):
    for name in names:
      copies[name].wait()

  def mod(i):
    return mod_v[0:1, i * d:(i + 1) * d]

  def normed(i):
    r = pl.ds(_aligned(i * _RB, _RB), _RB)
    return _layernorm(x_v[r, :].astype(_F32))

  def modulate(slot, xn):
    h_v[slot] = _pack(xn * (1.0 + mod(1)) + mod(0))

  def move_lanes(tiles, col, width):
    t, off = divmod(col, _LANES)
    if off == 0:
      return tiles[t]
    merged = tiles[t]
    if off + width > _LANES:
      lane = lax.broadcasted_iota(jnp.int32, merged.shape, 1)
      merged = jnp.where(lane >= off, merged, tiles[t + 1])
    return pltpu.roll(merged, _LANES - off, 1)

  def splat_keys(dst, pair, u, first, n, dims=range(_DH)):
    blocks = pl.ds(first, n)
    k = k_vpu[pair, blocks].reshape(n * _VK, _LANES)
    for i in dims:
      lane = u * _DH + i
      dst[blocks, pl.ds(i * _VK, _VK), :] = jnp.broadcast_to(
          k[:, lane:lane + 1], k.shape).reshape(n, _VK, _LANES)

  def project_k(i, slot):
    keys = _dot(_unpack(h_v[slot]), wqkv_v[:, d:2 * d])
    for jj in range(rb_steps):
      j = i * rb_steps + jj
      blocks = [keys[jj * _KB + n:jj * _KB + n + _VK]
                for n in range(0, _KB, _VK)]
      streamed = _pack(jnp.concatenate(blocks[:0:-1]))
      moves = [(streamed, k_mxu, j, 16), (blocks[0], k_vpu, j, 1)]
      if jj == 0:
        moves.append((blocks[_EXTRA], k_vpu, n_steps + j // _PERIOD, 1))
      for src, dst, at, align in moves:
        tiles = [src[:, t:t + _LANES] for t in range(0, d, _LANES)]
        for pair in range(n_pairs):
          skip = pair * pd % align
          dst[pair, at, 0:src.shape[0], :] = move_lanes(
              tiles, pair * pd - skip, pd + skip)

  def project_q(i, slot, lo=0, hi=d):
    q = _dot_nt(_unpack(wqv_t[lo // 2:hi // 2, :]), _unpack(h_v[slot]))
    q = q * (_DH ** -0.5 * math.log2(math.e))
    q_vpu[i, lo // pd:hi // pd, 0:pd] = q.reshape((hi - lo) // pd, pd, _RB)
    q_mxu[i, lo // 2:hi // 2] = _pack(q)

  def project_v(i, slot):
    lane = lax.broadcasted_iota(jnp.int32, (d, _KB), 1)
    low = lax.broadcasted_iota(jnp.int32, (8, _KB), 0) < 4
    v = _dot_nt(_unpack(wqv_t[d // 2:d, :]), _unpack(h_v[slot]))
    v = v.astype(_BF16).astype(_F32)
    for jj in range(rb_steps):
      j = i * rb_steps + jj
      natural = v[:, jj * _KB:(jj + 1) * _KB]
      shifted = pltpu.roll(natural, _KB - _VK, 1)
      for t in range(_NT):
        at = _VPU_AT[t] * _VK
        vt = natural if at == 0 else jnp.where(
            lane < at, shifted,
            jnp.where(lane < at + _VK, pltpu.roll(natural, at, 1), natural))
        for head in range(0, _HEADS, 2):
          r = head * _DH
          shared = vt[r + 16:r + 24]
          v_t[j, head, t, 0:16, :] = vt[r:r + 16]
          v_t[j, head, t, 16:24, :] = jnp.where(low, shared, 1.0)
          v_t[j, head + 1, t, 0:8, :] = jnp.where(low, 1.0, shared)
          v_t[j, head + 1, t, 8:24, :] = vt[r + 24:r + 40]

  start("c", "x0", "shift")
  for i in range(zeros_s.shape[0]):
    zeros_s[i] = 0
  unsafe_v[...] = jnp.zeros_like(unsafe_v)
  wd_v[f:, :] = jnp.zeros((wd_v.shape[0] - f, d), wd_v.dtype)
  wait("c")
  c = c_v[0].astype(_F32)
  silu_c = jnp.broadcast_to(c * jax.nn.sigmoid(c), (16, d)).astype(_BF16)
  wait("x0")
  start("scale")
  first_blocks = [normed(0), normed(1)]
  wait("shift")
  start("wk")
  mod_v[:, 0:d] = _dot(silu_c, wmod_v[:, 0:d])
  wait("scale")
  mod_v[:, d:2 * d] = _dot(silu_c, wmod_v[:, d:2 * d])
  start("wq")
  modulate(0, first_blocks[0])
  modulate(1, first_blocks[1])
  wait("wk")
  start("wv")
  project_k(0, 0)
  wait("wq")
  start("x1")
  project_k(1, 1)
  wqv_t[0:d // 2, :] = _pack(wqkv_v[:, 0:d].T)
  project_q(0, 0)
  splat_keys(splat_even, 0, 0, 0, 2 * rb_steps)
  wait("wv", "x1")
  start("x2")
  project_q(1, 1, 0, d // 2)
  wqv_t[d // 2:d, :] = _pack(wqkv_v[:, 2 * d:3 * d].T)
  project_v(0, 0)
  modulate(0, normed(2))
  project_v(1, 1)
  project_q(1, 1, d // 2, d)
  wait("x2")
  start(*late)

  @pl.loop(2, seq // _RB)
  def _(i):
    following = normed(jnp.minimum(i + 1, seq // _RB - 1))
    project_k(i, 0)
    project_v(i, 0)
    project_q(i, 0)
    modulate(0, following)
    splat_keys(splat_even, 0, 0, i * rb_steps, rb_steps)
    splat_keys(splat_even, 0, 0, n_steps + i * rb_steps // _PERIOD, 1)

  def masked_queries(pair, qb, u):
    skip = pair % 2 * 4
    at = pl.ds(_aligned(pair * _DH - skip + 8 * u, 8), 16)
    q = jnp.concatenate([q_mxu[2 * qb + n, at, :] for n in range(2)], axis=1)
    row = lax.broadcasted_iota(jnp.int32, q.shape, 0) + (8 * u - skip)
    mine = (row >= u * _DH // 2) & (row < (u + 1) * _DH // 2)
    parts = [jnp.zeros((8 * u, _QB), _U32), jnp.where(mine, q, _U32(0)),
             jnp.zeros((_LANES // 2 - 16 - 8 * u, _QB), _U32)]
    return _unpack(jnp.concatenate([p for p in parts if p.shape[0]]))

  def vpu_probs(unit, block, t, at=0, n=_VK):
    pair, qb, u = unit
    s = None
    for i in range(_DH):
      k = (splat_even, splat_odd)[u][block, pl.ds(i * _VK + at, n), :]
      q = q_vpu[2 * qb + t // 2, pair, pl.ds(u * _DH + i, 1),
                pl.ds(t % 2 * _LANES, _LANES)]
      term = k * jnp.broadcast_to(q, (n, _LANES))
      s = term if s is None else s + term
    return jnp.exp2(s)

  def extra_probs(unit, job):
    slot, part = divmod(job, _PERIOD)
    pair, qb, u = unit
    zero = zeros_s[job]
    p = vpu_probs((pair + zero, qb, u), n_steps + slot + zero, part // 2,
                  part % 2 * 8, 8)
    k_mxu[n_pairs + zeros_s[0], slot, pl.ds(8 * part, 8), :] = pltpu.bitcast(
        p, _U32)

  def mxu_probs(unit, following, queries, j):
    blocks = [(j, n) for n in range(_NB - 1, 0, -1)]
    if j % _PERIOD == _PERIOD - 2:
      blocks.remove((j, _EXTRA))
      blocks.append((j + 1, _NB - 1))
    elif j % _PERIOD == _PERIOD - 1:
      blocks = blocks[1:]
    k = []
    for at, (step, n) in enumerate(blocks):
      if at == _EXTRA_AT:
        extra_probs(unit if j + 1 < n_steps else following, (j + 1) % n_steps)
      k.append(k_mxu[unit[0], step, pl.ds(8 * (_NB - 1 - n), 8), :])
    p = jnp.exp2(_dot(_unpack(jnp.concatenate(k)), queries))
    return {block: p[at * _VK:(at + 1) * _VK]
            for at, block in enumerate(blocks)}

  def save_first(p):
    for (_, n), x in p.items():
      p_first[(n - 1) * _VK:n * _VK, :] = x

  def normalise(unit, acc):
    pair, qb, u = unit
    low = lax.broadcasted_iota(jnp.int32, (8, _QB), 0) < 4
    shared = acc[0:8] if u else acc[16:24]
    flipped = pltpu.roll(shared, 4, 0)
    total = (jnp.where(low, shared, flipped) if u else
             jnp.where(low, flipped, shared))
    inv = pl.reciprocal(total, approx=True)
    inv = inv * (2.0 - total * inv)
    o = [acc[n:n + 8] * inv for n in range(0, _VROWS, 8)]
    if u:
      o[0] = jnp.where(low, o_t[qb, pair, 16:24, :], o[0])
    o_t[qb, pair, pl.ds(16 * u, _VROWS), :] = jnp.concatenate(o)
    return o, total

  def finish(unit, acc):
    o, total = normalise(unit, acc)
    safe = ((total >= _SAFE_LO) & (total <= _SAFE_HI)
            & (jnp.abs(o[0] + o[1] + o[2]) < jnp.inf))
    unsafe_v[...] = jnp.where(safe, unsafe_v[...], 1.0)

  extra_probs((0, 0, 0), 0)
  save_first(mxu_probs((0, 0, 0), None, masked_queries(0, 0, 0), 0))

  @pl.loop(0, n_pairs)
  def _(pair):
    zero = [zeros_s[t] for t in range(_NT)]
    after = jnp.minimum(pair + 1, n_pairs - 1)

    def weighted_values(unit, j, p, saved):
      outs = []
      for t in range(_NT):
        blocks = [p[j, n][:, t * _LANES:(t + 1) * _LANES] if (j, n) in p
                  else saved[t] for n in range(1, _NB)]
        blocks.insert(_VPU_AT[t], vpu_probs(unit, j + zero[t], t))
        outs.append(_dot(v_t[j, 2 * pair + unit[2], t],
                         jnp.concatenate(blocks).astype(_BF16)))
      return jnp.concatenate(outs, axis=1)

    units = [(pair, qb, u) for u in range(2) for qb in range(n_qb)]
    units.append((after, 0, 0))
    p = {(0, n): p_first[(n - 1) * _VK:n * _VK, :] for n in range(1, _NB)}
    queries = masked_queries(*units[0])
    for unit, following in zip(units, units[1:]):
      _, qb, u = unit
      acc = None
      for j in range(n_steps):
        saved = None
        if j % _PERIOD == _PERIOD - 2:
          saved = [pltpu.bitcast(
              k_mxu[n_pairs + zero[2], j // _PERIOD, pl.ds(_VK * t, _VK), :],
              _F32) for t in range(_NT)]
        if j + 1 < n_steps:
          p.update(mxu_probs(unit, following, queries, j + 1))
          o = weighted_values(unit, j, p, saved)
          p = {block: x for block, x in p.items() if block[0] > j}
        else:
          queries = masked_queries(*following)
          p_following = mxu_probs(following, None, queries, 0)
          o = weighted_values(unit, j, p, saved)
          p = p_following
        acc = o if acc is None else acc + o
        part, dim = divmod(qb * n_steps + j, _DH)
        if part * _SPLAT < n_vpu:
          k_vpu[n_pairs + zero[0], 0, 0:8, :] = o[0:8, 0:_LANES]
          splat_keys(*((splat_even, after, 0) if u else (splat_odd, pair, 1)),
                     (part - 1) * _SPLAT % n_vpu, _SPLAT, (dim,))
      finish(unit, acc)
    save_first(p)

  def transpose_heads(b):
    o_v[...] = o_t[b].reshape(d, _QB).astype(_BF16).T

  wait(*late)
  transpose_heads(0)
  n_mod = 4 * d // sk
  for n in range(n_mod):
    for r in range(n * (fh // 16) // n_mod * 16,
                   (n + 1) * (fh // 16) // n_mod * 16, 16):
      for m, w in enumerate(_strassen_rhs_sums(*[
          wd_v[top + r:top + r + 16, left:left + sk]
          for top in (0, fh) for left in (0, sk)])):
        wd_sums[m, r:r + 16, :] = w
    at = pl.ds(2 * d + n * sk, sk)
    part = _dot(silu_c, wmod_v[:, at])
    mod_v[:, at] = part
    wd_v[pl.ds(pl.multiple_of(2 * fh + zeros_s[0], 16), 16), 0:_LANES] = (
        part[:, 0:_LANES].astype(wd_v.dtype))

  @pl.when(jnp.max(unsafe_v[...]) > 0.0)
  def _():
    @pl.loop(0, n_pairs * n_qb)
    def _(i):
      pair, qb = i // n_qb, i % n_qb
      for u in range(2):
        queries = masked_queries(pair, qb, u)

        def step(j, carry, u=u, queries=queries):
          m, acc = carry
          first = k_vpu[pair, j]
          first = jnp.where(pair % 2 == 1, pltpu.roll(first, 8, 1), first)
          rest = _dot(_unpack(k_mxu[pair, j, 0:(_KB - _VK) // 2, :]), queries)
          s = jnp.concatenate(
              [_dot(first.astype(_BF16), queries)]
              + [rest[n:n + _VK] for n in range(0, _KB - _VK, _VK)][::-1])
          m_new = jnp.maximum(m, jnp.max(s, axis=0, keepdims=True))
          p = jnp.exp2(s - m_new).astype(_BF16)
          o = _dot(v_t[j, 2 * pair + u, _VPU_AT.index(0)], p)
          return m_new, acc * jnp.exp2(m - m_new) + o

        init = (jnp.full((1, _QB), float(jnp.finfo(_F32).min), _F32),
                jnp.zeros((_VROWS, _QB), _F32))
        normalise((pair, qb, u), lax.fori_loop(0, n_steps, step, init)[1])

    transpose_heads(0)

  hm = _RB // 2

  def block_rows(b, half):
    return pl.ds(_aligned(b * _QB + half * _RB, _RB), _RB)

  def out_copy(b, half):
    r = block_rows(b, half)
    return pltpu.make_async_copy(
        out_v.at[r, :], out_hbm.at[r, :], out_sems.at[2 * b + half])

  def attention_residual(b, half):
    y = jnp.concatenate([
        _dot(o_v[r:r + _LANES, :], wo_v[...])
        for r in range(half * _RB, (half + 1) * _RB, _LANES)])
    x1 = x_v[block_rows(b, half), :].astype(_F32) + mod(2) * y
    h = _layernorm(x1) * (1.0 + mod(4)) + mod(3)
    return x1, h.astype(_BF16), _strassen_lhs(
        h[:hm, :sk], h[:hm, sk:2 * sk], h[hm:, :sk], h[hm:, sk:2 * sk])

  def geglu_tile(half, n, h, lhs):
    if n == f_main:
      both = _dot_nt(h, wgu_v[2 * f_main:2 * f, :])
      act = _gelu(both[:, 0:f_tail]) * both[:, f_tail:2 * f_tail]
      return jnp.concatenate(
          [act, jnp.zeros((_RB, _LANES - f_tail), _F32)], axis=1)
    gate_rows, up_rows = pl.ds(n, _LANES), pl.ds(f_main + n, _LANES)
    if half == 0:
      sums = _strassen_rhs_sums(*[
          wgu_v[at, left:left + sk]
          for left in (0, sk) for at in (gate_rows, up_rows)])
      for m, w in enumerate(sums):
        wgu_sums[m, gate_rows] = w
    else:
      sums = [wgu_sums[m, gate_rows] for m in range(5)]
    gate, up = _strassen(
        _dot_nt, lhs, sums, wgu_v[gate_rows, 0:sk], wgu_v[up_rows, sk:2 * sk],
        [_dot_nt(h[:, 2 * sk:], wgu_v[at, 2 * sk:])
         for at in (gate_rows, up_rows)])
    return _gelu(gate) * up

  def geglu(half, h, lhs):
    for n in range(0, fh, _LANES):
      left = geglu_tile(half, n, h, lhs)
      right = geglu_tile(half, fh + n, h, lhs)
      parts = _strassen_lhs(left[:hm], right[:hm], left[hm:], right[hm:])
      parts += [right[:hm].astype(_BF16), left[hm:].astype(_BF16)]
      for m, part in enumerate(parts):
        act_v[half, m, :, n:n + _LANES] = part

  def down(b, half, x1):
    lhs = [act_v[half, m] for m in range(9)]
    rest = jnp.concatenate([
        _dot(left, wd_v[0:fh, 2 * sk:]) + _dot(right, wd_v[fh:2 * fh, 2 * sk:])
        for left, right in ((lhs[2], lhs[7]), (lhs[8], lhs[3]))])
    y = _strassen(_dot, lhs, [wd_sums[m] for m in range(5)],
                  wd_v[0:fh, 0:sk], wd_v[fh:2 * fh, sk:2 * sk])
    out_v[block_rows(b, half), :] = (
        x1 + mod(5) * jnp.concatenate([*y, rest], axis=1)).astype(out_v.dtype)
    out_copy(b, half).start()

  @pl.loop(0, n_qb)
  def _(b):
    ready = [attention_residual(b, half) for half in range(2)]
    for half, (_, h, lhs) in enumerate(ready):
      geglu(half, h, lhs)
    down(b, 0, ready[0][0])
    transpose_heads(jnp.minimum(b + 1, n_qb - 1))
    down(b, 1, ready[1][0])

  for b in range(n_qb):
    for half in range(2):
      out_copy(b, half).wait()


@jax.jit
def pallas_adaLN_cond__mha_block__geglu_ffn__prompt_kernel(
    A_x: jax.Array,
    A_wqkv: jax.Array,
    A_wo: jax.Array,
    B_x: jax.Array,
    B_w_gate: jax.Array,
    B_w_up: jax.Array,
    B_w_down: jax.Array,
    c: jax.Array,
    w_mod: jax.Array,
):
  del B_x
  batch, seq, d = A_x.shape
  f = B_w_down.shape[0]
  assert batch == 1 and d == _HEADS * _DH
  n_qb, n_rb, n_steps = seq // _QB, seq // _RB, seq // _KB
  n_vpu = n_steps + n_steps // _PERIOD
  n_pairs = _HEADS // 2
  f_main = f // _LANES * _LANES
  fh = (f_main + _LANES) // 2

  vmem = pltpu.VMEM
  scratch_shapes = [
      vmem((seq, d), A_x.dtype),
      vmem(A_wqkv.shape, A_wqkv.dtype),
      vmem(A_wo.shape, A_wo.dtype),
      vmem((2 * f, d), B_w_gate.dtype),
      vmem((2 * fh + 64, d), B_w_down.dtype),
      vmem(w_mod.shape, w_mod.dtype),
      vmem((32,) + c.shape, c.dtype),
      vmem((seq, d), A_x.dtype),
      vmem((16, 6 * d), _F32),
      vmem((d, d), _U32),
      vmem((2, _RB // 2, d), _U32),
      vmem((n_pairs + 1, n_steps, _KB // 2, _LANES), _U32),
      vmem((n_pairs + 1, n_vpu, _VK, _LANES), _F32),
      vmem((n_vpu, _DH * _VK, _LANES), _F32),
      vmem((n_vpu, _DH * _VK, _LANES), _F32),
      vmem((n_rb, d // 2, _RB), _U32),
      vmem((n_rb, n_pairs, 48, _RB), _F32),
      vmem((n_steps, _HEADS, _NT, _VROWS, _KB), _F32),
      vmem((_KB - _VK, _QB), _F32),
      vmem((n_qb, n_pairs, 2 * _DH, _QB), _F32),
      vmem((8, _QB), _F32),
      vmem((_QB, d), _BF16),
      vmem((2, 9, _RB // 2, fh), _BF16),
      vmem((5, f_main, _STRASSEN_K), _BF16),
      vmem((5, fh, _STRASSEN_K), _BF16),
      pltpu.SMEM((n_steps,), jnp.int32),
      pltpu.SemaphoreType.DMA((16,)),
      pltpu.SemaphoreType.DMA((n_rb,)),
  ]
  out = pl.pallas_call(
      _kernel,
      out_shape=jax.ShapeDtypeStruct((seq, d), A_x.dtype),
      in_specs=[pl.BlockSpec(memory_space=pltpu.HBM)] * 8,
      out_specs=pl.BlockSpec(memory_space=pltpu.HBM),
      scratch_shapes=scratch_shapes,
      compiler_params=pltpu.CompilerParams(
          vmem_limit_bytes=120 * 1024 * 1024),
      name="adaln_mha_geglu",
  )(A_x.reshape(seq, d), A_wqkv, A_wo, B_w_gate.T, B_w_up.T, B_w_down, c,
    w_mod)
  return out.reshape(batch, seq, d)
```

```python
import math

import jax
import jax.numpy as jnp
from jax import lax
import jax.experimental.pallas as pl
import jax.experimental.pallas.tpu as pltpu

_HEADS = 32
_DH = 20
_LANES = 128
_QB = 512
_NT = _QB // _LANES
_RB = _QB // 2
_KB = 128
_VK = 16
_NB = _KB // _VK
_VROWS = 24
_VPU_AT = (0, 2, 5, 7)
_PERIOD = 8
_EXTRA = 5
_EXTRA_AT = 5
_SPLAT = 6
_STRASSEN_K = 2 * _LANES
_EPS = 1e-5
_SAFE_LO = 2.0 ** -60
_SAFE_HI = 2.0 ** 60

_F32 = jnp.float32
_BF16 = jnp.bfloat16
_U32 = jnp.uint32


def _dot(a, b):
  return jnp.dot(a, b, preferred_element_type=_F32)


def _dot_nt(a, b):
  return lax.dot_general(a, b, (((1,), (1,)), ((), ())),
                         preferred_element_type=_F32)


def _pack(x):
  return pltpu.bitcast(x.astype(_BF16), _U32)


def _unpack(x):
  return pltpu.bitcast(x, _BF16)


def _aligned(i, n):
  return i if isinstance(i, int) else pl.multiple_of(i, n)


def _layernorm(x):
  mean = jnp.mean(x, axis=-1, keepdims=True)
  centred = x - mean
  var = jnp.mean(centred * centred, axis=-1, keepdims=True)
  return centred * lax.rsqrt(var + _EPS)


def _gelu(x):
  c = math.sqrt(2.0 / math.pi)
  half = 0.5 * x
  return half + half * jnp.tanh(x * (c + (c * 0.044715) * (x * x)))


def _strassen_lhs(a11, a12, a21, a22):
  return [a.astype(_BF16) for a in (
      a11 + a22, a21 + a22, a11, a22, a11 + a12, a21 - a11, a12 - a22)]


def _strassen_rhs_sums(b11, b12, b21, b22):
  b11, b12, b21, b22 = [b.astype(_F32) for b in (b11, b12, b21, b22)]
  return [b.astype(_BF16) for b in (
      b11 + b22, b12 - b22, b21 - b11, b11 + b12, b21 + b22)]


def _strassen(dot, lhs, sums, b11, b22, init=None):
  rhs = [sums[0], b11, sums[1], sums[2], b22, sums[3], sums[4]]
  signs = ((1, 0, 0, 1), (0, 0, 1, -1), (0, 1, 0, 1), (1, 0, 1, 0),
           (-1, 1, 0, 0), (0, 0, 0, 1), (1, 0, 0, 0))
  c = [None] * 4
  if init is not None:
    c = [q for row in zip(*[jnp.split(x, 2) for x in init]) for q in row]
  for n in (2, 4, 1, 3, 0, 6, 5):
    m = dot(lhs[n], rhs[n])
    for i, sign in enumerate(signs[n]):
      if sign and c[i] is None:
        c[i] = m if sign > 0 else -m
      elif sign:
        c[i] = c[i] + m if sign > 0 else c[i] - m
  return jnp.concatenate([c[0], c[2]]), jnp.concatenate([c[1], c[3]])


def _kernel(
    x_hbm, wqkv_hbm, wo_hbm, wg_hbm, wu_hbm, wd_hbm, c_hbm, wmod_hbm, out_hbm,
    x_v, wqkv_v, wo_v, wgu_v, wd_v, wmod_v, c_v, out_v,
    mod_v, wqv_t, h_v, k_mxu, k_vpu, splat_even, splat_odd, q_mxu, q_vpu, v_t,
    p_first, o_t, unsafe_v, o_v, act_v, wgu_sums, wd_sums, zeros_s,
    sems, out_sems):
  seq, d = x_v.shape
  f = wd_hbm.shape[0]
  n_qb = seq // _QB
  n_steps = seq // _KB
  n_vpu = n_steps + n_steps // _PERIOD
  rb_steps = _RB // _KB
  n_pairs = _HEADS // 2
  pd = 2 * _DH
  sk = _STRASSEN_K
  fh = wd_sums.shape[1]
  fm = fh - _LANES
  ht = _LANES // 2
  n_tails = (f - 2 * fm) // ht

  def cols(src, dst, lo, hi):
    return src.at[:, pl.ds(lo, hi - lo)], dst.at[:, pl.ds(lo, hi - lo)]

  def rows(src, dst, lo, hi, to=None):
    return (src.at[pl.ds(lo, hi - lo), :],
            dst.at[pl.ds(lo if to is None else to, hi - lo), :])

  pieces = dict(
      c=(c_hbm, c_v.at[0]),
      x0=rows(x_hbm, x_v, 0, _QB),
      shift=cols(wmod_hbm, wmod_v, 0, d),
      scale=cols(wmod_hbm, wmod_v, d, 2 * d),
      wk=cols(wqkv_hbm, wqkv_v, d, 2 * d),
      wq=cols(wqkv_hbm, wqkv_v, 0, d),
      wv=cols(wqkv_hbm, wqkv_v, 2 * d, 3 * d),
      x1=rows(x_hbm, x_v, _QB, _QB + _RB),
      x2=rows(x_hbm, x_v, _QB + _RB, seq),
      mod=cols(wmod_hbm, wmod_v, 2 * d, 6 * d),
      wo=(wo_hbm, wo_v),
      wg=rows(wg_hbm, wgu_v, 0, 2 * fm),
      wu=rows(wu_hbm, wgu_v, 0, 2 * fm, 2 * fm),
      wd0=rows(wd_hbm, wd_v, 0, fm),
      wd1=rows(wd_hbm, wd_v, fm, 2 * fm, fh),
      wd2=rows(wd_hbm, wd_v, 2 * fm, fm + fh, fm),
      wd3=rows(wd_hbm, wd_v, fm + fh, f),
  )
  for n in range(n_tails):
    for half, w in enumerate((wg_hbm, wu_hbm)):
      pieces[f"tail{n}{half}"] = rows(
          w, wgu_v, 2 * fm + n * ht, 2 * fm + (n + 1) * ht,
          4 * fm + (2 * n + half) * ht)
  late = list(pieces)[list(pieces).index("mod"):]
  copies = {name: pltpu.make_async_copy(src, dst, sems.at[i])
            for i, (name, (src, dst)) in enumerate(pieces.items())}

  def start(*names):
    for name in names:
      copies[name].start()

  def wait(*names):
    for name in names:
      copies[name].wait()

  def mod(i):
    return mod_v[0:1, i * d:(i + 1) * d]

  def normed(i):
    r = pl.ds(_aligned(i * _RB, _RB), _RB)
    return _layernorm(x_v[r, :].astype(_F32))

  def modulate(slot, xn):
    h_v[slot] = _pack(xn * (1.0 + mod(1)) + mod(0))

  def move_lanes(tiles, col, width):
    t, off = divmod(col, _LANES)
    if off == 0:
      return tiles[t]
    merged = tiles[t]
    if off + width > _LANES:
      lane = lax.broadcasted_iota(jnp.int32, merged.shape, 1)
      merged = jnp.where(lane >= off, merged, tiles[t + 1])
    return pltpu.roll(merged, _LANES - off, 1)

  def splat_keys(dst, pair, u, first, n, dims=range(_DH)):
    blocks = pl.ds(first, n)
    k = k_vpu[pair, blocks].reshape(n * _VK, _LANES)
    for i in dims:
      lane = u * _DH + i
      dst[blocks, pl.ds(i * _VK, _VK), :] = jnp.broadcast_to(
          k[:, lane:lane + 1], k.shape).reshape(n, _VK, _LANES)

  def project_k(i, slot):
    keys = _dot(_unpack(h_v[slot]), wqkv_v[:, d:2 * d])
    for jj in range(rb_steps):
      j = i * rb_steps + jj
      blocks = [keys[jj * _KB + n:jj * _KB + n + _VK]
                for n in range(0, _KB, _VK)]
      streamed = _pack(jnp.concatenate(blocks[:0:-1]))
      moves = [(streamed, k_mxu, j, 16), (blocks[0], k_vpu, j, 1)]
      if jj == 0:
        moves.append((blocks[_EXTRA], k_vpu, n_steps + j // _PERIOD, 1))
      for src, dst, at, align in moves:
        tiles = [src[:, t:t + _LANES] for t in range(0, d, _LANES)]
        for pair in range(n_pairs):
          skip = pair * pd % align
          dst[pair, at, 0:src.shape[0], :] = move_lanes(
              tiles, pair * pd - skip, pd + skip)

  def project_q(i, slot, lo=0, hi=d):
    q = _dot_nt(_unpack(wqv_t[lo // 2:hi // 2, :]), _unpack(h_v[slot]))
    q = q * (_DH ** -0.5 * math.log2(math.e))
    q_vpu[i, lo // pd:hi // pd, 0:pd] = q.reshape((hi - lo) // pd, pd, _RB)
    q_mxu[i, lo // 2:hi // 2] = _pack(q)

  def project_v(i, slot):
    lane = lax.broadcasted_iota(jnp.int32, (d, _KB), 1)
    low = lax.broadcasted_iota(jnp.int32, (8, _KB), 0) < 4
    v = _dot_nt(_unpack(wqv_t[d // 2:d, :]), _unpack(h_v[slot]))
    for jj in range(rb_steps):
      j = i * rb_steps + jj
      natural = v[:, jj * _KB:(jj + 1) * _KB]
      shifted = pltpu.roll(natural, _KB - _VK, 1)
      for t in range(_NT):
        at = _VPU_AT[t] * _VK
        vt = natural if at == 0 else shifted if at == _KB - _VK else jnp.where(
            lane < at, shifted,
            jnp.where(lane < at + _VK, pltpu.roll(natural, at, 1), natural))
        for head in range(0, _HEADS, 2):
          r = head * _DH
          shared = vt[r + 16:r + 24]
          v_t[j, head, t, 0:16, :] = vt[r:r + 16]
          v_t[j, head, t, 16:24, :] = jnp.where(low, shared, 1.0)
          v_t[j, head + 1, t, 0:8, :] = jnp.where(low, 1.0, shared)
          v_t[j, head + 1, t, 8:24, :] = vt[r + 24:r + 40]

  start("c", "x0", "shift")
  for i in range(zeros_s.shape[0]):
    zeros_s[i] = 0
  unsafe_v[...] = jnp.zeros_like(unsafe_v)
  wd_v[f:, :] = jnp.zeros((wd_v.shape[0] - f, d), wd_v.dtype)
  wait("c")
  c = c_v[0].astype(_F32)
  silu_c = jnp.broadcast_to(c * jax.nn.sigmoid(c), (16, d)).astype(_BF16)
  wait("x0")
  start("scale")
  first_blocks = [normed(0), normed(1)]
  wait("shift")
  start("wk")
  mod_v[:, 0:d] = _dot(silu_c, wmod_v[:, 0:d])
  wait("scale")
  mod_v[:, d:2 * d] = _dot(silu_c, wmod_v[:, d:2 * d])
  start("wq")
  modulate(0, first_blocks[0])
  modulate(1, first_blocks[1])
  wait("wk")
  start("wv")
  project_k(0, 0)
  wait("wq")
  start("x1")
  project_k(1, 1)
  wqv_t[0:d // 2, :] = _pack(wqkv_v[:, 0:d].T)
  project_q(0, 0)
  splat_keys(splat_even, 0, 0, 0, 2 * rb_steps)
  wait("wv", "x1")
  start("x2")
  project_q(1, 1, 0, d // 2)
  wqv_t[d // 2:d, :] = _pack(wqkv_v[:, 2 * d:3 * d].T)
  project_v(0, 0)
  modulate(0, normed(2))
  project_v(1, 1)
  project_q(1, 1, d // 2, d)
  wait("x2")
  start(*late)

  @pl.loop(2, seq // _RB)
  def _(i):
    following = normed(jnp.minimum(i + 1, seq // _RB - 1))
    project_k(i, 0)
    project_v(i, 0)
    project_q(i, 0)
    modulate(0, following)
    splat_keys(splat_even, 0, 0, i * rb_steps, rb_steps)
    splat_keys(splat_even, 0, 0, n_steps + i * rb_steps // _PERIOD, 1)

  def masked_queries(pair, qb, u):
    skip = pair % 2 * 4
    at = pl.ds(_aligned(pair * _DH - skip + 8 * u, 8), 16)
    q = jnp.concatenate([q_mxu[2 * qb + n, at, :] for n in range(2)], axis=1)
    row = lax.broadcasted_iota(jnp.int32, q.shape, 0) + (8 * u - skip)
    mine = (row >= u * _DH // 2) & (row < (u + 1) * _DH // 2)
    parts = [jnp.zeros((8 * u, _QB), _U32), jnp.where(mine, q, _U32(0)),
             jnp.zeros((_LANES // 2 - 16 - 8 * u, _QB), _U32)]
    return _unpack(jnp.concatenate([p for p in parts if p.shape[0]]))

  def vpu_probs(unit, block, t, at=0, n=_VK):
    pair, qb, u = unit
    s = None
    for i in range(_DH):
      k = (splat_even, splat_odd)[u][block, pl.ds(i * _VK + at, n), :]
      q = q_vpu[2 * qb + t // 2, pair, pl.ds(u * _DH + i, 1),
                pl.ds(t % 2 * _LANES, _LANES)]
      term = k * jnp.broadcast_to(q, (n, _LANES))
      s = term if s is None else s + term
    return jnp.exp2(s)

  def extra_probs(unit, job):
    slot, part = divmod(job, _PERIOD)
    pair, qb, u = unit
    zero = zeros_s[job]
    p = vpu_probs((pair + zero, qb, u), n_steps + slot + zero, part // 2,
                  part % 2 * 8, 8)
    k_mxu[n_pairs + zeros_s[0], slot, pl.ds(8 * part, 8), :] = pltpu.bitcast(
        p, _U32)

  def mxu_probs(unit, following, queries, j):
    blocks = [(j, n) for n in range(_NB - 1, 0, -1)]
    if j % _PERIOD == _PERIOD - 2:
      blocks.remove((j, _EXTRA))
      blocks.append((j + 1, _NB - 1))
    elif j % _PERIOD == _PERIOD - 1:
      blocks = blocks[1:]
    k = []
    for at, (step, n) in enumerate(blocks):
      if at == _EXTRA_AT:
        extra_probs(unit if j + 1 < n_steps else following, (j + 1) % n_steps)
      k.append(k_mxu[unit[0], step, pl.ds(8 * (_NB - 1 - n), 8), :])
    p = jnp.exp2(_dot(_unpack(jnp.concatenate(k)), queries))
    return {block: p[at * _VK:(at + 1) * _VK]
            for at, block in enumerate(blocks)}

  def save_first(p):
    for (_, n), x in p.items():
      p_first[(n - 1) * _VK:n * _VK, :] = x

  def normalise(unit, acc):
    pair, qb, u = unit
    low = lax.broadcasted_iota(jnp.int32, (8, _QB), 0) < 4
    shared = acc[0:8] if u else acc[16:24]
    flipped = pltpu.roll(shared, 4, 0)
    total = (jnp.where(low, shared, flipped) if u else
             jnp.where(low, flipped, shared))
    inv = pl.reciprocal(total, approx=True)
    inv = inv * (2.0 - total * inv)
    o = [acc[n:n + 8] * inv for n in range(0, _VROWS, 8)]
    if u:
      o[0] = jnp.where(low, o_t[qb, pair, 16:24, :], o[0])
    o_t[qb, pair, pl.ds(16 * u, _VROWS), :] = jnp.concatenate(o)
    return o, total

  def finish(unit, acc):
    o, total = normalise(unit, acc)
    safe = ((total >= _SAFE_LO) & (total <= _SAFE_HI)
            & (jnp.abs(o[0] + o[1] + o[2]) < jnp.inf))
    unsafe_v[...] = jnp.where(safe, unsafe_v[...], 1.0)

  extra_probs((0, 0, 0), 0)
  save_first(mxu_probs((0, 0, 0), None, masked_queries(0, 0, 0), 0))

  @pl.loop(0, n_pairs)
  def _(pair):
    zero = [zeros_s[t] for t in range(_NT)]
    after = jnp.minimum(pair + 1, n_pairs - 1)

    def weighted_values(unit, j, p, saved):
      outs = []
      for t in range(_NT):
        blocks = [p[j, n][:, t * _LANES:(t + 1) * _LANES] if (j, n) in p
                  else saved[t] for n in range(1, _NB)]
        blocks.insert(_VPU_AT[t], vpu_probs(unit, j + zero[t], t))
        outs.append(_dot(v_t[j, 2 * pair + unit[2], t],
                         jnp.concatenate(blocks).astype(_BF16)))
      return jnp.concatenate(outs, axis=1)

    units = [(pair, qb, u) for u in range(2) for qb in range(n_qb)]
    units.append((after, 0, 0))
    p = {(0, n): p_first[(n - 1) * _VK:n * _VK, :] for n in range(1, _NB)}
    queries = masked_queries(*units[0])
    for unit, following in zip(units, units[1:]):
      _, qb, u = unit
      acc = None
      for j in range(n_steps):
        saved = None
        if j % _PERIOD == _PERIOD - 2:
          saved = [pltpu.bitcast(
              k_mxu[n_pairs + zero[2], j // _PERIOD, pl.ds(_VK * t, _VK), :],
              _F32) for t in range(_NT)]
        if j + 1 < n_steps:
          p.update(mxu_probs(unit, following, queries, j + 1))
          o = weighted_values(unit, j, p, saved)
          p = {block: x for block, x in p.items() if block[0] > j}
        else:
          queries = masked_queries(*following)
          p_following = mxu_probs(following, None, queries, 0)
          o = weighted_values(unit, j, p, saved)
          p = p_following
        acc = o if acc is None else acc + o
        part, dim = divmod(qb * n_steps + j, _DH)
        if part * _SPLAT < n_vpu:
          k_vpu[n_pairs + zero[0], 0, 0:8, :] = o[0:8, 0:_LANES]
          splat_keys(*((splat_even, after, 0) if u else (splat_odd, pair, 1)),
                     (part - 1) * _SPLAT % n_vpu, _SPLAT, (dim,))
      finish(unit, acc)
    save_first(p)

  def transpose_heads(b):
    o_v[...] = o_t[b].reshape(d, _QB).astype(_BF16).T

  wait(*late)
  transpose_heads(0)
  n_mod = 4 * d // sk
  for n in range(n_mod):
    for r in range(n * (fh // 16) // n_mod * 16,
                   (n + 1) * (fh // 16) // n_mod * 16, 16):
      for m, w in enumerate(_strassen_rhs_sums(*[
          wd_v[top + r:top + r + 16, left:left + sk]
          for top in (0, fh) for left in (0, sk)])):
        wd_sums[m, r:r + 16, :] = w
    at = pl.ds(2 * d + n * sk, sk)
    part = _dot(silu_c, wmod_v[:, at])
    mod_v[:, at] = part
    wd_v[pl.ds(pl.multiple_of(2 * fh + zeros_s[0], 16), 16), 0:_LANES] = (
        part[:, 0:_LANES].astype(wd_v.dtype))

  for r in range(0, _LANES, 16):
    for m, w in enumerate(_strassen_rhs_sums(*[
        wgu_v[top + r:top + r + 16, left:left + sk]
        for left in (0, sk) for top in (0, fm)])):
      wgu_sums[m, r:r + 16, :] = w

  @pl.when(jnp.max(unsafe_v[...]) > 0.0)
  def _():
    @pl.loop(0, n_pairs * n_qb)
    def _(i):
      pair, qb = i // n_qb, i % n_qb
      for u in range(2):
        queries = masked_queries(pair, qb, u)

        def step(j, carry, u=u, queries=queries):
          m, acc = carry
          first = k_vpu[pair, j]
          first = jnp.where(pair % 2 == 1, pltpu.roll(first, 8, 1), first)
          rest = _dot(_unpack(k_mxu[pair, j, 0:(_KB - _VK) // 2, :]), queries)
          s = jnp.concatenate(
              [_dot(first.astype(_BF16), queries)]
              + [rest[n:n + _VK] for n in range(0, _KB - _VK, _VK)][::-1])
          m_new = jnp.maximum(m, jnp.max(s, axis=0, keepdims=True))
          p = jnp.exp2(s - m_new).astype(_BF16)
          o = _dot(v_t[j, 2 * pair + u, _VPU_AT.index(0)], p)
          return m_new, acc * jnp.exp2(m - m_new) + o

        init = (jnp.full((1, _QB), float(jnp.finfo(_F32).min), _F32),
                jnp.zeros((_VROWS, _QB), _F32))
        normalise((pair, qb, u), lax.fori_loop(0, n_steps, step, init)[1])

    transpose_heads(0)

  hm = _RB // 2

  def block_rows(b, half):
    return pl.ds(_aligned(b * _QB + half * _RB, _RB), _RB)

  def out_copy(b, half):
    r = block_rows(b, half)
    return pltpu.make_async_copy(
        out_v.at[r, :], out_hbm.at[r, :], out_sems.at[2 * b + half])

  def attention_residual(b, half):
    y = jnp.concatenate([
        _dot(o_v[r:r + _LANES, :], wo_v[...])
        for r in range(half * _RB, (half + 1) * _RB, _LANES)])
    x1 = x_v[block_rows(b, half), :].astype(_F32) + mod(2) * y
    h = _layernorm(x1) * (1.0 + mod(4)) + mod(3)
    return x1, h.astype(_BF16), _strassen_lhs(
        h[:hm, :sk], h[:hm, sk:2 * sk], h[hm:, :sk], h[hm:, sk:2 * sk])

  def hidden(half, h, lhs, first, second):
    tiles = pl.ds(first, _LANES), pl.ds(second, _LANES)
    if half == 0 and first > 0:
      sums = _strassen_rhs_sums(*[
          wgu_v[at, left:left + sk] for left in (0, sk) for at in tiles])
      for m, w in enumerate(sums):
        wgu_sums[m, tiles[0]] = w
    else:
      sums = [wgu_sums[m, tiles[0]] for m in range(5)]
    return _strassen(
        _dot_nt, lhs, sums, wgu_v[tiles[0], 0:sk], wgu_v[tiles[1], sk:2 * sk],
        [_dot_nt(h[:, 2 * sk:], wgu_v[at, 2 * sk:]) for at in tiles])

  def geglu(half, h, lhs):
    for n in range(0, fh, _LANES):
      if n < fm:
        gate = hidden(half, h, lhs, n, fm + n)
        up = hidden(half, h, lhs, 2 * fm + n, 3 * fm + n)
        left, right = [_gelu(g) * u for g, u in zip(gate, up)]
      else:
        tails = [*hidden(half, h, lhs, 4 * fm, 4 * fm + _LANES),
                 _dot_nt(h, wgu_v[4 * fm + 2 * _LANES:, :])]
        tails = [_gelu(x[:, :ht]) * x[:, ht:] for x in tails]
        left = jnp.concatenate(tails[:2], axis=1)
        right = jnp.concatenate([tails[2], jnp.zeros_like(tails[2])], axis=1)
      parts = _strassen_lhs(left[:hm], right[:hm], left[hm:], right[hm:])
      parts += [right[:hm].astype(_BF16), left[hm:].astype(_BF16)]
      for m, part in enumerate(parts):
        act_v[half, m, :, n:n + _LANES] = part

  def down(b, half, x1):
    lhs = [act_v[half, m] for m in range(9)]
    rest = jnp.concatenate([
        _dot(left, wd_v[0:fh, 2 * sk:]) + _dot(right, wd_v[fh:2 * fh, 2 * sk:])
        for left, right in ((lhs[2], lhs[7]), (lhs[8], lhs[3]))])
    y = _strassen(_dot, lhs, [wd_sums[m] for m in range(5)],
                  wd_v[0:fh, 0:sk], wd_v[fh:2 * fh, sk:2 * sk])
    out_v[block_rows(b, half), :] = (
        x1 + mod(5) * jnp.concatenate([*y, rest], axis=1)).astype(out_v.dtype)
    out_copy(b, half).start()

  @pl.loop(0, n_qb)
  def _(b):
    ready = [attention_residual(b, half) for half in range(2)]
    for half, (_, h, lhs) in enumerate(ready):
      geglu(half, h, lhs)
    down(b, 0, ready[0][0])
    transpose_heads(jnp.minimum(b + 1, n_qb - 1))
    down(b, 1, ready[1][0])

  for b in range(n_qb):
    for half in range(2):
      out_copy(b, half).wait()


@jax.jit
def pallas_adaLN_cond__mha_block__geglu_ffn__prompt_kernel(
    A_x: jax.Array,
    A_wqkv: jax.Array,
    A_wo: jax.Array,
    B_x: jax.Array,
    B_w_gate: jax.Array,
    B_w_up: jax.Array,
    B_w_down: jax.Array,
    c: jax.Array,
    w_mod: jax.Array,
):
  del B_x
  batch, seq, d = A_x.shape
  f = B_w_down.shape[0]
  assert batch == 1 and d == _HEADS * _DH
  n_qb, n_rb, n_steps = seq // _QB, seq // _RB, seq // _KB
  n_vpu = n_steps + n_steps // _PERIOD
  n_pairs = _HEADS // 2
  fh = pl.cdiv(f, 2 * _LANES) * _LANES
  assert 2 * fh - f == _LANES // 2

  vmem = pltpu.VMEM
  scratch_shapes = [
      vmem((seq, d), A_x.dtype),
      vmem(A_wqkv.shape, A_wqkv.dtype),
      vmem(A_wo.shape, A_wo.dtype),
      vmem((2 * f, d), B_w_gate.dtype),
      vmem((2 * fh + 64, d), B_w_down.dtype),
      vmem(w_mod.shape, w_mod.dtype),
      vmem((32,) + c.shape, c.dtype),
      vmem((seq, d), A_x.dtype),
      vmem((16, 6 * d), _F32),
      vmem((d, d), _U32),
      vmem((2, _RB // 2, d), _U32),
      vmem((n_pairs + 1, n_steps, _KB // 2, _LANES), _U32),
      vmem((n_pairs + 1, n_vpu, _VK, _LANES), _F32),
      vmem((n_vpu, _DH * _VK, _LANES), _F32),
      vmem((n_vpu, _DH * _VK, _LANES), _F32),
      vmem((n_rb, d // 2, _RB), _U32),
      vmem((n_rb, n_pairs, 48, _RB), _F32),
      vmem((n_steps, _HEADS, _NT, _VROWS, _KB), _F32),
      vmem((_KB - _VK, _QB), _F32),
      vmem((n_qb, n_pairs, 2 * _DH, _QB), _F32),
      vmem((8, _QB), _F32),
      vmem((_QB, d), _BF16),
      vmem((2, 9, _RB // 2, fh), _BF16),
      vmem((5, 4 * fh, _STRASSEN_K), _BF16),
      vmem((5, fh, _STRASSEN_K), _BF16),
      pltpu.SMEM((n_steps,), jnp.int32),
      pltpu.SemaphoreType.DMA((23,)),
      pltpu.SemaphoreType.DMA((n_rb,)),
  ]
  out = pl.pallas_call(
      _kernel,
      out_shape=jax.ShapeDtypeStruct((seq, d), A_x.dtype),
      in_specs=[pl.BlockSpec(memory_space=pltpu.HBM)] * 8,
      out_specs=pl.BlockSpec(memory_space=pltpu.HBM),
      scratch_shapes=scratch_shapes,
      compiler_params=pltpu.CompilerParams(
          vmem_limit_bytes=120 * 1024 * 1024),
      name="adaln_mha_geglu",
  )(A_x.reshape(seq, d), A_wqkv, A_wo, B_w_gate.T, B_w_up.T, B_w_down, c,
    w_mod)
  return out.reshape(batch, seq, d)
```
